```python
import os as _os
_os.environ.setdefault("JAX_PLATFORMS", "cpu")
import jax
import jax.numpy as jnp

def _softmax(x, axis=-1):
    return jax.nn.softmax(x, axis=axis)
def _gelu(x):
    return jax.nn.gelu(x, approximate=True)
def _silu(x):
    return jax.nn.silu(x)
def _sigmoid(x):
    return jax.nn.sigmoid(x)
def _layernorm(x, axis=-1, eps=1e-5):
    m = jnp.mean(x, axis=axis, keepdims=True)
    v = jnp.var(x, axis=axis, keepdims=True)
    return (x - m) / jnp.sqrt(v + eps)
def _scatter_add(tgt, idx, src, axis=0):
    return tgt.at[idx].add(src)
def _segment_sum(src, seg, n):
    return jax.ops.segment_sum(src, seg, n)
class _Rng:
    def __init__(self, key):
        self._k = key
    def _next(self):
        self._k, sub = jax.random.split(self._k)
        return sub
    def normal(self, shape):
        return jax.random.normal(self._next(), shape, dtype=jnp.bfloat16)
    def randint(self, lo, hi, shape):
        return jax.random.randint(self._next(), shape, lo, hi, dtype=jnp.int32)
    def uniform(self, shape, lo=0.0, hi=1.0):
        return jax.random.uniform(self._next(), shape, jnp.bfloat16, lo, hi)
    def permutation(self, n):
        return jax.random.permutation(self._next(), n)


kernel_name = 'interleave_layers__sliding_local_dilated__moe_arch_mod__prompt'

def setup_inputs():
    _rng = _Rng(jax.random.key(int.from_bytes(__import__("os").urandom(4), "little")))
    _w = (lambda a: (lambda t: t.astype(jnp.bfloat16) if jnp.issubdtype(t.dtype, jnp.floating) else t)(jnp.asarray(a)))
    def _A_setup():
        B, S, D = 1, 2048, 512
        return {
            "x": _w((lambda *s: _rng.normal(s) * 0.05)(B, S, D)),
            "wqkv": _w((lambda *s: _rng.normal(s) * 0.05)(D, 3 * D)),
            "wo": _w((lambda *s: _rng.normal(s) * 0.05)(D, D)),
        }
    _A_in = _A_setup()

    def _B_setup():
        B, S, D, F, C = 1, 2048, 512, 1376, 2
        return {
            "x": _w((lambda *s: _rng.normal(s) * 0.05)(B, S, D)),
            "w_r": _w((lambda *s: _rng.normal(s) * 0.05)(D)),
            "w_gate": _w((lambda *s: _rng.normal(s) * 0.05)(D, F)),
            "w_up": _w((lambda *s: _rng.normal(s) * 0.05)(D, F)),
            "w_down": _w((lambda *s: _rng.normal(s) * 0.05)(F, D)),
        }
    _B_in = _B_setup()

    return {
        "A_x": _A_in["x"],
        "A_wqkv": _A_in["wqkv"],
        "A_wo": _A_in["wo"],
        "B_x": _B_in["x"],
        "B_w_r": _B_in["w_r"],
        "B_w_gate": _B_in["w_gate"],
        "B_w_up": _B_in["w_up"],
        "B_w_down": _B_in["w_down"],
    }

def reference(A_x, A_wqkv, A_wo, B_x, B_w_r, B_w_gate, B_w_up, B_w_down):
    def _A_ref(x, wqkv, wo):
        B, S, D = x.shape
        H = 32; Dh = D // H
        W, dil = 8, 2
        qkv = (lambda x, *d: x.transpose(*d))((x @ wqkv).reshape(B, S, 3, H, Dh), 2, 0, 3, 1, 4)
        q, k, v = qkv[0], qkv[1], qkv[2]
        scale = Dh ** -0.5
        pos = jnp.arange(S)
        off = jnp.arange(W) * dil
        idx = pos[:, None] - off[None, :]
        mask = idx >= 0
        idx_c = jnp.where(mask, idx, 0).reshape(-1)
        kg = k[:, :, idx_c, :].reshape(B, H, S, W, Dh)
        vg = v[:, :, idx_c, :].reshape(B, H, S, W, Dh)
        logits = jnp.einsum("bhsd,bhswd->bhsw", q, kg) * scale
        logits = jnp.where(mask[None, None, :, :], logits, -1e9)
        attn = _softmax(logits, axis=-1)
        o = jnp.einsum("bhsw,bhswd->bhsd", attn, vg)
        return (lambda x, *d: x.transpose(*d))(o, 0, 2, 1, 3).reshape(B, S, D) @ wo

    def _B_ref(x, w_r, w_gate, w_up, w_down):
        B, S, D = x.shape
        C = 2
        r = x @ w_r
        idx = jnp.argsort(-r, axis=-1)[:, :C]
        idx_e = jnp.repeat(idx.reshape(B, C, 1), D, axis=2)
        x_sel = jnp.take_along_axis(x, idx_e, axis=1)
        g = _silu(x_sel @ w_gate)
        u = x_sel @ w_up
        y = (g * u) @ w_down
        r_sel = _sigmoid(jnp.take_along_axis(r, idx, axis=1))
        y = y * r_sel.reshape(B, C, 1)
        b_off = (jnp.arange(B) * S).reshape(B, 1)
        flat_idx = (idx + b_off).reshape(B * C)
        zero = (x * 0.0).reshape(B * S, D)
        upd = _scatter_add(zero, flat_idx, y.reshape(B * C, D), axis=0)
        return x + upd.reshape(B, S, D)

    x = A_x
    x = x + _A_ref(_layernorm(x, axis=-1), A_wqkv, A_wo)
    x = x + _B_ref(_layernorm(x, axis=-1), B_w_r, B_w_gate, B_w_up, B_w_down)
    x = x + _A_ref(_layernorm(x, axis=-1), A_wqkv, A_wo)
    x = x + _B_ref(_layernorm(x, axis=-1), B_w_r, B_w_gate, B_w_up, B_w_down)
    return x
```

```python
import jax
import jax.numpy as jnp
from jax import lax
import jax.experimental.pallas as pl
import jax.experimental.pallas.tpu as pltpu

S, D, F = 2048, 512, 1376
NJ = 8
EPS = 1e-5
NEG = -999292928.0
F32, BF16, U32, I32 = jnp.float32, jnp.bfloat16, jnp.uint32, jnp.int32
NT = (((1,), (1,)), ((), ()))
TN = (((0,), (0,)), ((), ()))


def _pack(x):
    return pltpu.bitcast(x.astype(BF16), U32)


def _unpack(u):
    return pltpu.bitcast(u, BF16)


def _rb(x):
    return x.astype(BF16).astype(F32)


def _center(x):
    m = jnp.sum(x, axis=0, keepdims=True) * (1.0 / D)
    c = x - m
    v = jnp.sum(c * c, axis=0, keepdims=True) * (1.0 / D)
    return c, 1.0 / _rb(jnp.sqrt(_rb(_rb(v) + EPS)))


def _kernel(x_hbm, wqkv_hbm, wo_hbm, wr_ref, wg_hbm, wu_hbm, wd_hbm, out_hbm,
            xin, xout, wqkv, wo, wg, wu, wd, wt, wot, wrc,
            x0, x1, xn0, xn1, xb, k0, v0, k1, v1, v00, qa, qb, oa, ob, r_ref, sems):
    xs, xns, ks, vs = (x0, x1), (xn0, xn1), (k0, k1), (v0, v1)
    qs, os_ = (qa, qb), (oa, ob)
    lane = lax.broadcasted_iota(I32, (8, 128), 1)

    def x_copy(sb, c):
        return pltpu.make_async_copy(
            x_hbm.at[pl.ds(1024 * sb, 1024), pl.ds(128 * c, 128)],
            xin.at[c, pl.ds(1024 * sb, 1024)], sems.at[4 * sb + c])

    def w_copy(t):
        return pltpu.make_async_copy(
            wqkv_hbm.at[:, pl.ds(512 * t, 512)], wqkv.at[t], sems.at[8 + t])

    def o_copy(sb, c):
        return pltpu.make_async_copy(
            xout.at[c, pl.ds(1024 * sb, 1024)],
            out_hbm.at[pl.ds(1024 * sb, 1024), pl.ds(128 * c, 128)], sems.at[4 * sb + c])

    wo_copy = pltpu.make_async_copy(wo_hbm, wo, sems.at[11])
    ffn_copies = [pltpu.make_async_copy(a, b, sems.at[12 + i])
                  for i, (a, b) in enumerate(((wg_hbm, wg), (wu_hbm, wu), (wd_hbm, wd)))]

    w_copy(1).start()
    for c in range(4):
        x_copy(0, c).start()
    w_copy(2).start()
    w_copy(0).start()
    wo_copy.start()
    for c in range(4):
        x_copy(1, c).start()
    for cp in ffn_copies:
        cp.start()

    ri = lax.broadcasted_iota(I32, (128, 128), 0)
    ci = lax.broadcasted_iota(I32, (128, 128), 1)
    perm = jnp.where(ci == (ri % 8) * 16 + ri // 8, 1.0, 0.0).astype(BF16)
    perm_t = jnp.where(ri == (ci % 8) * 16 + ci // 8, 1.0, 0.0).astype(BF16)

    def prep_w(t):
        w_copy(t).wait()
        for g in range(4):
            w = lax.dot_general(perm, wqkv[t, :, pl.ds(128 * g, 128)], NT,
                                preferred_element_type=F32)
            wt[t, pl.ds(64 * g, 64), :] = _pack(w)

    def prep_wo():
        wo_copy.wait()
        for g in range(4):
            w = lax.dot_general(wo[pl.ds(128 * g, 128), :], perm_t, TN,
                                preferred_element_type=F32)
            wot[:, pl.ds(128 * g, 128)] = _pack(w)
        wrc[...] = jnp.broadcast_to(wr_ref[...].astype(F32).reshape(1, D), (128, D)).T

    xin_u = xin.bitcast(U32)
    xout_u = xout.bitcast(U32)

    def ln_store(sb, j, x):
        c, rs = _center(x)
        xns[sb][j] = _pack(c * rs)

    def prep_in(sb, j):
        parts = []
        for c in range(4):
            u = xin_u[c, pl.ds(512 * sb + j, 64, stride=8), :]
            parts.append(_unpack(u).T.astype(F32))
        x = jnp.concatenate(parts, axis=0)
        xs[sb][j] = x
        ln_store(sb, j, x)

    def prep_mid(sb, j):
        ln_store(sb, j, xs[sb][j])

    def proj(t, sb, j):
        return jnp.dot(_unpack(wt[t]), _unpack(xns[sb][j]), preferred_element_type=F32)

    def kv(sb, j):
        rhs = _unpack(xns[sb][j])
        kvw = jnp.concatenate([_unpack(wt[1]), _unpack(wt[2])], axis=0)
        r = jnp.dot(kvw, rhs, preferred_element_type=F32)
        k, v = r[:D], r[D:]
        ks[sb][NJ + j] = k
        vs[sb][NJ + j] = v
        lane_f = lax.broadcasted_iota(I32, (D, 128), 1)
        if sb == 0 and j == 0:
            v00[...] = jnp.where(lane_f == 0, v, pltpu.roll(v, 1, 1))
        if j > 0:
            if sb == 0:
                k0[j] = pltpu.roll(k, 2, 1)
                v0[j] = jnp.where(lane_f < 2, v00[...], pltpu.roll(v, 2, 1))
            else:
                k1[j] = jnp.where(lane_f < 2, k0[j], pltpu.roll(k, 2, 1))
                v1[j] = pltpu.roll(jnp.where(lane_f >= 126, v0[NJ + j], v), 2, 1)

    def qproj(sb, j):
        qs[j % 2][...] = proj(0, sb, j)

    def attn(sb, j):
        q_ref, o_ref, k_ref, v_ref = qs[j % 2], os_[j % 2], ks[sb], vs[sb]
        for g in range(4):
            acc = [None] * NJ
            for d in range(16):
                rows = pl.ds(128 * g + 8 * d, 8)
                q = q_ref[rows, :]
                for w in range(NJ):
                    p = q * k_ref[NJ + j - w, rows, :]
                    acc[w] = p if d == 0 else acc[w] + p
            acc = [a * 0.25 for a in acc]
            if sb == 0:
                for w in range(j + 1, NJ):
                    acc[w] = jnp.where(lane < 2, NEG, acc[w])
            m = acc[0]
            for w in range(1, NJ):
                m = jnp.maximum(m, acc[w])
            e = [jnp.exp(a - m) for a in acc]
            den = e[0]
            for w in range(1, NJ):
                den = den + e[w]
            inv = 1.0 / den
            p = [a * inv for a in e]
            for d2 in range(8):
                halves = []
                for d in (2 * d2, 2 * d2 + 1):
                    rows = pl.ds(128 * g + 8 * d, 8)
                    o = p[0] * v_ref[NJ + j, rows, :]
                    for w in range(1, NJ):
                        o = o + p[w] * v_ref[NJ + j - w, rows, :]
                    halves.append(o)
                o_ref[pl.ds(64 * g + 8 * d2, 8), :] = _pack(jnp.concatenate(halves, axis=0))

    def oproj(sb, j, last):
        x = xs[sb][j] + jnp.dot(_unpack(wot[...]), _unpack(os_[j % 2][...]),
                                preferred_element_type=F32)
        c, rs = _center(x)
        xn = c * rs
        n = NJ * sb + j
        r_ref[pl.ds(n, 1), :] = jnp.sum(xn * wrc[...], axis=0, keepdims=True)
        xb[n] = _pack(xn)
        y = x + xn
        if last:
            yb = y.astype(BF16)
            for cc in range(4):
                xout_u[cc, pl.ds(512 * sb + j, 64, stride=8), :] = pltpu.bitcast(
                    yb[128 * cc:128 * cc + 128].T, U32)
        else:
            xs[sb][j] = y

    def route():
        r = r_ref[...]
        blk = lax.broadcasted_iota(I32, (16, 128), 0)
        ln = lax.broadcasted_iota(I32, (16, 128), 1)
        tok = (blk // 8) * 1024 + (ln // 2) * 16 + (blk % 8) * 2 + ln % 2
        tokf = tok.astype(F32)
        key = jnp.where(r != r, -jnp.inf, r)
        m1 = jnp.max(key, keepdims=True)
        i1 = jnp.min(jnp.where(key == m1, tokf, 4096.0), keepdims=True)
        key2 = jnp.where(tokf == i1, -jnp.inf, key)
        m2 = jnp.max(key2, keepdims=True)
        i2 = jnp.min(jnp.where((key2 == m2) & (tokf != i1), tokf, 4096.0), keepdims=True)
        r1 = jnp.sum(jnp.where(tokf == i1, r, 0.0), keepdims=True)
        r2 = jnp.sum(jnp.where(tokf == i2, r, 0.0), keepdims=True)
        toks = [i1.astype(I32)[0, 0], i2.astype(I32)[0, 0]]
        row = lax.broadcasted_iota(I32, (16, 128), 0)
        lane_u = lax.broadcasted_iota(I32, (D // 2, 128), 1)
        xsel = None
        locs = []
        for i, t in enumerate(toks):
            t = jnp.clip(t, 0, S - 1)
            sb, j = t // 1024, (t // 2) % 8
            ln_i = ((t % 1024) // 16) * 2 + t % 2
            locs.append((t, sb, j, ln_i))
            col = jnp.where(lane_u == ln_i, xb[NJ * sb + j], jnp.uint32(0))
            sel = jnp.where(row == i, 1.0, 0.0).astype(BF16)
            part = lax.dot_general(sel, _unpack(col), NT, preferred_element_type=F32)
            xsel = part if xsel is None else xsel + part
        xsel = xsel.astype(BF16)
        g = lax.dot_general(xsel, wg[...], NT, preferred_element_type=F32)
        u = lax.dot_general(xsel, wu[...], NT, preferred_element_type=F32)
        h = (g * jax.nn.sigmoid(g) * u).astype(BF16)
        y = jnp.dot(h, wd[...], preferred_element_type=F32)
        ys = [y[0:1] * jax.nn.sigmoid(r1), y[1:2] * jax.nn.sigmoid(r2)]
        return locs, ys

    def scatter_mid(locs, ys):
        lane_f = lax.broadcasted_iota(I32, (D, 128), 1)
        for (t, sb, j, ln_i), y in zip(locs, ys):
            col = jnp.broadcast_to(y, (128, D)).T
            for s in range(2):
                @pl.when(sb == s)
                def _():
                    cur = xs[s][j]
                    xs[s][j] = jnp.where(lane_f == ln_i, cur + col, cur)

    def scatter_out(locs, ys):
        row = lax.broadcasted_iota(I32, (16, 128), 0)
        bases = []
        for (t, sb, j, ln_i), y in zip(locs, ys):
            base = pl.multiple_of((t // 16) * 16, 16)
            bases.append(base)
            for c in range(4):
                cur = xout[c, pl.ds(base, 16), :].astype(F32)
                new = jnp.where(row == t % 16, cur + y[:, 128 * c:128 * c + 128], cur)
                xout[c, pl.ds(base, 16), :] = new.astype(BF16)

        def patch(i, c):
            return pltpu.make_async_copy(
                xout.at[c, pl.ds(bases[i], 16)],
                out_hbm.at[pl.ds(bases[i], 16), pl.ds(128 * c, 128)], sems.at[4 * i + c])

        for c in range(4):
            patch(0, c).start()

        @pl.when(bases[0] != bases[1])
        def _():
            for c in range(4):
                patch(1, c).start()
            for c in range(4):
                patch(1, c).wait()

        for c in range(4):
            patch(0, c).wait()

    prep_w(1)
    for c in range(4):
        x_copy(0, c).wait()
    prep_in(0, 0)
    prep_w(2)

    for layer in range(2):
        last = layer == 1
        prep = prep_mid if last else prep_in
        if last:
            prep(0, 0)
        for j in range(NJ):
            kv(0, j)
            if j + 1 < NJ:
                prep(0, j + 1)
        if not last:
            prep_w(0)
            prep_wo()
            for c in range(4):
                x_copy(1, c).wait()
        prep(1, 0)
        qproj(0, 0)
        for n in range(2 * NJ):
            sb, j = divmod(n, NJ)
            if sb == 0:
                kv(1, j)
                if j + 1 < NJ:
                    prep(1, j + 1)
            if n > 0:
                oproj(*divmod(n - 1, NJ), last)
            if n + 1 < 2 * NJ:
                qproj(*divmod(n + 1, NJ))
            attn(sb, j)
            if last and n == NJ:
                for c in range(4):
                    o_copy(0, c).start()
        oproj(1, NJ - 1, last)
        if not last:
            for cp in ffn_copies:
                cp.wait()
            scatter_mid(*route())
        else:
            for c in range(4):
                o_copy(1, c).start()
            locs, ys = route()
            for sb in range(2):
                for c in range(4):
                    o_copy(sb, c).wait()
            scatter_out(locs, ys)


@jax.jit
def pallas_interleave_layers__sliding_local_dilated__moe_arch_mod__prompt_kernel(
    A_x, A_wqkv, A_wo, B_x, B_w_r, B_w_gate, B_w_up, B_w_down,
):
    del B_x
    hbm = pl.BlockSpec(memory_space=pl.ANY)
    V = pltpu.VMEM
    scratch = [
        V((4, S, 128), BF16), V((4, S, 128), BF16),
        V((3, D, D), BF16), V((D, D), BF16),
        V((F, D), BF16), V((F, D), BF16), V((F, D), BF16),
        V((3, D // 2, D), U32), V((D // 2, D), U32), V((D, 128), F32),
        V((NJ, D, 128), F32), V((NJ, D, 128), F32),
        V((NJ, D // 2, 128), U32), V((NJ, D // 2, 128), U32),
        V((2 * NJ, D // 2, 128), U32),
        V((2 * NJ, D, 128), F32), V((2 * NJ, D, 128), F32),
        V((2 * NJ, D, 128), F32), V((2 * NJ, D, 128), F32),
        V((D, 128), F32),
        V((D, 128), F32), V((D, 128), F32),
        V((D // 2, 128), U32), V((D // 2, 128), U32),
        V((2 * NJ, 128), F32),
        pltpu.SemaphoreType.DMA((16,)),
    ]
    out = pl.pallas_call(
        _kernel,
        out_shape=jax.ShapeDtypeStruct((S, D), BF16),
        in_specs=[hbm, hbm, hbm, pl.BlockSpec(memory_space=pltpu.VMEM), hbm, hbm, hbm],
        out_specs=hbm,
        scratch_shapes=scratch,
        compiler_params=pltpu.CompilerParams(vmem_limit_bytes=64 * 1024 * 1024),
    )(A_x.reshape(S, D), A_wqkv, A_wo, B_w_r, B_w_gate.T, B_w_up.T, B_w_down)
    return out.reshape(1, S, D)
```

```python
import jax
import jax.numpy as jnp
from jax import lax
import jax.experimental.pallas as pl
import jax.experimental.pallas.tpu as pltpu

S, D, F = 2048, 512, 1376
FP = 1408
NJ = 8
NB = 2 * NJ
EPS = 1e-5
NEG = -1e9
F32, BF16, U32, I32 = jnp.float32, jnp.bfloat16, jnp.uint32, jnp.int32
NT = (((1,), (1,)), ((), ()))
SLAB = 32
R = 64

DENSE, LIGHT = "dense", "light"
FIRST = (
    LIGHT, ("S0",), ("X0 R0",), ("S1",), ("W1 K0", "X1 R1 ."), ("K1",), ("S2",), ("W2 V1",), ("S3",),
    ("V0", "X2 R2 ."), ("K2 V2", "X3 R3 X4 R4 ."), ("K3 V3", "X5 R5 X6 R6 X7 ."), ("K4",), ("S4",),
    ("V4 K5 V5 W0", "W3 X8 X9 X10 X11 X12 X13 X14 X15"))
SHARED = (
    LIGHT, ("V6 K6", "R7 R8 ."), ("V7", "R9"), ("K7 Q0", "C0"), ("B8 Q1", "R10", "A0"),
    ("B9 Q2 O0", "R11", "A1"), ("B10 Q3 O1", "R12 P0", "A2"), ("B11 Q4 O2", "R13 P1", "A3"),
    ("B12 Q5 O3", "R14 P2", "A4"), ("B13 Q6 O4", "R15 P3", "A5"), ("B14 Q7 O5", "P4", "A6"),
    ("B15 Q8 O6", "P5", "A7"))
MIDDLE = (
    DENSE, ("U0 U1",), ("Q9 O7", "P6 A8"), ("Q10 O8", "P7 A9"), ("S0",), ("Q11 O9", "P8 A10"),
    ("Q12 O10", "P9 A11"),
    LIGHT, ("Q13 O11 K0", "R0 P10", "A12"), ("Q14 O12 V0", "P11 R1", "A13"), ("S1",),
    ("Q15 O13 K1", "P12 R2", "A14"), ("O14 V1", "P13 R3", "A15"), ("K2 O15", "P14"), ("V2", "P15 ."),
    ("K3", "R4"), ("V3",), ("S2",), ("K4", "R5"), ("S3",), ("S4",), ("V4",), ("S5",), ("K5 V5", "R6 ."))
LAST = (
    DENSE, ("Q9 O7", "P6 A8"), ("Q10 O8", "P7 A9"), ("S0",), ("Q11 O9", "P8 A10"), ("Q12 O10", "P9 A11"),
    ("Q13 O11 Q14", "A12 A13"), ("O12 Q15", "P10 A14"), ("O13 O14", "A15 P11 P12"), ("O15", "P13 P14"),
    ("P15",), ("S1",), ("S2",), ("S3",), ("S4",), ("S5",))
COST = dict(idle=0.4, qk=16, sm=48, pv=31, p1=40, p2=40, p3=20, r1=8, r2=24, r3=30, r4=12)


def _unpack(u):
    return pltpu.bitcast(u, BF16)


def _fold(x):
    parts = [x[8 * i:8 * i + 8] for i in range(x.shape[0] // 8)]
    while len(parts) > 1:
        parts = [parts[i] + parts[i + 1] for i in range(0, len(parts), 2)]
    return parts[0]


def _acc(a, b):
    return b if a is None else a + b


def _mean(partial):
    return jnp.sum(partial, axis=0, keepdims=True) * (1.0 / D)


def _rows(row):
    return jnp.broadcast_to(row, (R, 128))


def _once(fn):
    def gen():
        fn()
        yield 0
    return gen(), 0


def _interleave(streams):
    def chain(tasks):
        for gen, _ in tasks:
            yield from gen
    live = [[chain(t), 0, max(1, sum(c for _, c in t))] for t in reversed(streams)]
    while live:
        st = min(live, key=lambda e: e[1] / e[2])
        cost = next(st[0], None)
        if cost is None:
            live = [e for e in live if e is not st]
        else:
            st[1] += cost


def _kernel(x_hbm, x3_hbm, wqkv_hbm, wo_hbm, wr_hbm, wg_hbm, wu_hbm, wd_hbm, out_hbm,
            xhead, xin, xout, wqkv, wo, wr, wg, wu, wd, wt, wot, wrc, wgu,
            xr, xo, xq, xn, xc, kv, qs, os_, ca, v00, stat, r_ref, sems, idle_sem):
    zero = pl.semaphore_read(idle_sem)
    pace = dict(token=None, seen=set(), light=True, due=[])

    def fence(ref, val):
        if val.dtype != ref.dtype:
            val = pltpu.bitcast(val, ref.dtype)
        mid = tuple(n - 1 for n in ref.shape[1:-2])
        ref[(zero,) + mid + (pl.ds(ref.shape[-2] - 8, 8), pl.ds(0, 128))] = val

    def tick(val):
        pace["token"] = val
        pace["seen"].clear()

    def gate(ref, after=None):
        val = None if id(ref) in pace["seen"] else pace["token"]
        if after is not None and pace["light"]:
            val = _acc(val, after)
        if val is not None:
            fence(ref, val)
            pace["seen"].add(id(ref))

    def copies(pairs, sem0):
        return [pltpu.make_async_copy(a, b, sems.at[sem0 + i]) for i, (a, b) in enumerate(pairs)]

    def tiles(c):
        return pl.ds(128 * c, 128)

    def half(s):
        return pl.ds(S // 2 * s, S // 2)

    x_cp = [copies([(x_hbm.at[half(s), tiles(c)], xin.at[c, half(s)]) for c in range(4)], 4 * s)
            for s in range(2)]
    head_cp = copies([(x3_hbm.at[pl.ds(0, 64), pl.ds(2 * j, 2)], xhead.at[:, pl.ds(2 * j, 2)])
                      for j in range(2)], 8)
    w_cp = copies([(wqkv_hbm.at[:, pl.ds(D * t, D)], wqkv.at[t]) for t in range(3)], 10)
    wo_cp = copies([(wo_hbm.at[:, tiles(c)], wo.at[c]) for c in range(4)] + [(wr_hbm, wr)], 13)
    ffn_cp = copies([(wg_hbm, wg), (wu_hbm, wu), (wd_hbm, wd)], 18)

    def out_cp(s, z=0):
        return copies([(xout.at[c + z, half(s)], out_hbm.at[half(s), tiles(c)]) for c in range(4)], 4 * s)

    def dma(start=(), wait=()):
        def run():
            for cp in start:
                cp.start()
            for cp in wait:
                cp.wait()
            if wait:
                tick(None)
        return run

    def layout_qkv(t):
        def gen():
            a = lax.broadcasted_iota(I32, (128, 128), 0)
            b = lax.broadcasted_iota(I32, (128, 128), 1)
            perm = jnp.where(b == (a % 8) * 16 + a // 8, 0.25 if t == 0 else 1.0, 0.0).astype(BF16)
            for g in range(4):
                w = lax.dot_general(perm, wqkv[t, :, tiles(g)], NT, preferred_element_type=F32)
                wt[t][0, pl.ds(64 * g, 64), :] = pltpu.bitcast(w.astype(BF16), U32)
                tick(w[-8:, -128:])
                if g == 3:
                    fence(wt[t], pace["token"])
                yield 128
        return gen(), 512

    def layout_out():
        def gen():
            wrc[0, pl.ds(0, D), :] = jnp.broadcast_to(
                wr[...].astype(F32).reshape(1, D), (128, D)).astype(BF16).T.astype(F32)
            for c in range(4):
                for g in range(4):
                    rows = []
                    for d2 in range(8):
                        u = wo.bitcast(U32)[c, pl.ds(64 * g + d2, 8, stride=8), :]
                        rows += [u << 16, u & jnp.uint32(0xFFFF0000)]
                    w = pltpu.bitcast(jnp.concatenate(rows, axis=0), F32)
                    w = pltpu.bitcast(w.astype(BF16).T, U32)
                    for ref in wot:
                        ref[0, pl.ds(64 * c, 64), tiles(g)] = w
                    yield 32
        return gen(), 512

    def layout_ffn(i):
        def run():
            for f in range(FP // 128):
                rows = min(128, F - 128 * f)
                for c in range(4):
                    w = (wg, wu)[i][pl.ds(128 * f, rows), tiles(c)]
                    if rows < 128:
                        w = jnp.concatenate([w, jnp.zeros((128 - rows, 128), BF16)], axis=0)
                    wgu[i, pl.ds(64 * c, 64), tiles(f)] = pltpu.bitcast(w.T, U32)
        return _once(run)

    def block_rows(n):
        return pl.ds(S // 4 * (n // NJ) + n % NJ, 64, stride=NJ)

    def load_x(n):
        cost = 128 if n < 2 else 24

        def gen():
            for c in range(4):
                if n < 2:
                    u = xhead.bitcast(U32)[:, n, tiles(c)]
                else:
                    u = xin.bitcast(U32)[c, block_rows(n), :]
                xr[0, n, tiles(c), :] = _unpack(u).T.astype(F32)
                yield cost
        return gen(), 4 * cost

    def norm(i, n):
        def gen():
            s = None
            for r0 in range(0, D, R):
                gate(xr)
                s = _acc(s, _fold(xr[0, n, pl.ds(r0, R), :]))
                yield COST["r1"]
            m, s = _rows(_mean(s)), None
            for r0 in range(0, D, R):
                gate(xr, m[:8] if r0 == R else None)
                c = xr[0, n, pl.ds(r0, R), :] - m
                ca[0, pl.ds(r0, R), :] = c
                s = _acc(s, _fold(c * c))
                yield COST["r2"]
            rs = _rows(lax.rsqrt(_mean(s) + EPS))
            yield COST["r3"]
            for r0 in range(0, D, R):
                gate(ca, rs[:8] if r0 == R else None)
                y = ca[0, pl.ds(r0, R), :] * rs
                xn[i % NJ][0, pl.ds(r0, R), :] = y
                if i < NJ:
                    xq[0, n, pl.ds(r0, R), :] = y
                if r0 + R == D:
                    fence(xn[i % NJ], rs[:8])
                yield COST["r4"]
        return gen(), 8 * (COST["r1"] + COST["r2"] + COST["r4"]) + COST["r3"]

    def project(weights, ref, idx, store, done=None, reuse=False):
        m = D * len(weights)

        def gen():
            lhs = jnp.concatenate([w[0, pl.ds(0, D // 2), :] for w in weights], axis=0)
            rhs = ref[idx + (pl.ds(0, D), slice(None))].astype(BF16)
            out = jnp.dot(_unpack(lhs), rhs, preferred_element_type=F32)
            for r0 in range(0, m, SLAB):
                store(r0, out[r0:r0 + SLAB])
                tick(out[r0 + SLAB - 8:r0 + SLAB])
                if r0 == 0:
                    fence(ref, pace["token"])
                if (r0 + SLAB) % D == 0 and not reuse:
                    fence(weights[r0 // D], pace["token"])
                if done and r0 + SLAB == m:
                    done()
                yield SLAB
        return gen(), m

    def project_kv(i, j, lo, hi, reuse=False):
        s = i // NJ

        def store(r0, val):
            lane = lax.broadcasted_iota(I32, val.shape, 1)
            is_v = lo + r0 // D
            rows, off = pl.ds(r0 % D, SLAB), NB * is_v
            kv[s][0, off + NJ + j, rows, :] = val
            if isinstance(j, int) and j == 0:
                return
            if s == 0:
                shifted = pltpu.roll(val, 2, 1)
            elif is_v:
                shifted = pltpu.roll(jnp.where(lane >= 126, kv[0][0, off + NJ + j, rows, :], val), 2, 1)
            else:
                shifted = jnp.where(lane < 2, kv[0][0, j, rows, :], pltpu.roll(val, 2, 1))
            kv[s][0, off + j, rows, :] = shifted
        return project(wt[1 + lo:1 + hi], xn[i % NJ], (0,), store, reuse=reuse)

    def clamp_v(_):
        def gen():
            lane = lax.broadcasted_iota(I32, (R, 128), 1)
            for r0 in range(0, D, R):
                v = kv[0][0, NB + NJ, pl.ds(r0, R), :]
                v00[0, pl.ds(r0, R), :] = jnp.where(lane == 0, v, pltpu.roll(v, 1, 1))
            yield 120
            for r0 in range(0, D, R):
                gate(v00)
                v = v00[0, pl.ds(r0, R), :]
                for j in range(1, NJ):
                    pltpu.store(kv[0].at[0, NB + j, pl.ds(r0, R), :], v, mask=lane < 2)
                yield 60
        return gen(), 600

    def project_q(n):
        def store(r0, q):
            qs[n % 3][0, pl.ds(r0, SLAB), :] = q
        ref, idx = (xq, (0, n)) if n < NJ else (xn[n - NJ], (0,))
        return project(wt[:1], ref, idx, store, lambda: fence(qs[n % 3], pace["token"]))

    def attend(n):
        s, j = divmod(n, NJ)

        def gen():
            lane = lax.broadcasted_iota(I32, (8, 128), 1)
            for g in range(4):
                logit = [None] * NJ
                for d in range(16):
                    rows = pl.ds(128 * g + 8 * d, 8)
                    gate(kv[s])
                    q = qs[n % 3][0, rows, :]
                    for w in range(NJ):
                        logit[w] = _acc(logit[w], q * kv[s][0, NJ + j - w, rows, :])
                    yield COST["qk"]
                if s == 0:
                    for w in range(j + 1, NJ):
                        logit[w] = jnp.where(lane < 2, NEG, logit[w])
                top = logit
                while len(top) > 1:
                    top = [jnp.maximum(top[i], top[i + 1]) for i in range(0, len(top), 2)]
                e = [jnp.exp(a - top[0]) for a in logit]
                den = ((e[0] + e[1]) + (e[2] + e[3])) + ((e[4] + e[5]) + (e[6] + e[7]))
                inv = 1.0 / den
                yield COST["sm"]
                for d in range(16):
                    rows = pl.ds(128 * g + 8 * d, 8)
                    if d % 2 == 0:
                        gate(kv[s], den if d == 2 else None)
                    o = None
                    for w in range(NJ):
                        o = _acc(o, e[w] * kv[s][0, NB + NJ + j - w, rows, :])
                    os_[n % 3][0, rows, :] = o * inv
                    if (g, d) == (3, 15):
                        while pace["due"]:
                            o = o + pace["due"].pop()
                        fence(os_[n % 3], o)
                    if d % 2:
                        yield COST["pv"]
        return gen(), 4 * (16 * COST["qk"] + COST["sm"] + 8 * COST["pv"])

    def project_o(n):
        total = [None]

        def store(r0, y):
            x = xr[0, n, pl.ds(r0, SLAB), :] + y
            xo[n % 6][0, pl.ds(r0, SLAB), :] = x
            total[0] = _acc(total[0], _fold(x))

        def done():
            stat[NB + n % 6] = jnp.broadcast_to(_mean(total[0]), (8, 128))
        return project([wot[n % 2]], os_[n % 3], (0,), store, done)

    def post(n, keep, emit):
        def gen():
            m = jnp.concatenate([stat[NB + n % 6]] * (R // 8), axis=0)
            s = t = None
            for r0 in range(0, D, R):
                rows = pl.ds(r0, R)
                gate(xo[n % 6], m[:8] if r0 == R else None)
                c = xo[n % 6][0, rows, :] - m
                xc[0, n, rows, :] = c
                s = _acc(s, _fold(c * c))
                t = _acc(t, _fold(c * wrc[0, rows, :]))
                yield COST["p1"]
            rs = lax.rsqrt(_mean(s) + EPS)
            r_ref[pl.ds(n, 1), :] = jnp.sum(t, axis=0, keepdims=True) * rs
            stat[n] = jnp.broadcast_to(rs, (8, 128))
            fence(wrc, t)
            gain = _rows(rs + 1.0)
            yield COST["p2"]
            for c in range(4):
                gate(xc, gain[:8] if c == 1 else None)
                ys = []
                for r0 in range(128 * c, 128 * c + 128, R):
                    ys.append(xc[0, n, pl.ds(r0, R), :] * gain + m)
                    if keep:
                        xr[0, n, pl.ds(r0, R), :] = ys[-1]
                    yield COST["p3"]
                if emit:
                    y = jnp.concatenate(ys, axis=0).astype(BF16)
                    xout.bitcast(U32)[c, block_rows(n), :] = pltpu.bitcast(y.T, U32)
            if emit and n < 11:
                seen = xout.bitcast(U32)[zero + 3, pl.ds(S // 4 * (n // NJ) + n % NJ, 1), :]
                pace["due"].append(pltpu.bitcast(seen, F32))
        return gen(), 8 * (COST["p1"] + COST["p3"]) + COST["p2"]

    def top2(blocks):
        r = r_ref[pl.ds(0, blocks), :]
        blk = lax.broadcasted_iota(I32, r.shape, 0)
        lane = lax.broadcasted_iota(I32, r.shape, 1)
        tid = ((blk // NJ) * 1024 + (lane // 2) * 16 + (blk % NJ) * 2 + lane % 2).astype(F32)
        none = float(2 * S)
        key = jnp.where(r != r, -jnp.inf, r)
        best = key == jnp.max(key, keepdims=True)
        first = jnp.min(jnp.where(best, tid, none), keepdims=True)
        tied = jnp.sum(jnp.where(best, 1.0, 0.0), keepdims=True) > 1.5
        runner = jnp.max(jnp.where(best, -jnp.inf, key), keepdims=True)
        second = jnp.min(jnp.where(tied, jnp.where(best & (tid != first), tid, none),
                                   jnp.where(~best & (key == runner), tid, none)), keepdims=True)
        toks = [jnp.clip(i.astype(I32)[0, 0], 0, S - 1) for i in (first, second)]
        return toks, [jnp.sum(jnp.where(tid == i, r, 0.0), keepdims=True) for i in (first, second)]

    def locate(t):
        return (t // 1024) * NJ + (t // 2) % NJ, ((t % 1024) // 16) * 2 + t % 2

    def route_stages(st):
        def gather():
            st["toks"], st["scores"] = top2(NB)
            row = lax.broadcasted_iota(I32, (16, 128), 0)
            lane = lax.broadcasted_iota(I32, (D, 128), 1)
            sel = None
            for i, t in enumerate(st["toks"]):
                n, at = locate(t)
                col = jnp.where(lane == at, xc[0, n] * stat[n][:1], 0.0).astype(BF16)
                pick = jnp.where(row == i, 1.0, 0.0).astype(BF16)
                sel = _acc(sel, lax.dot_general(pick, col, NT, preferred_element_type=F32))
            st["x"] = sel.astype(BF16)

        def up():
            g, u = [jnp.dot(st["x"], _unpack(wgu[i, pl.ds(0, D // 2), :]),
                            preferred_element_type=F32)[:8, :F] for i in range(2)]
            h = g * jax.nn.sigmoid(g) * u
            st["h"] = jnp.concatenate([h, h], axis=0).astype(BF16)

        def down():
            y = jnp.dot(st["h"], wd[...], preferred_element_type=F32)
            st["y"] = [y[i:i + 1] * jax.nn.sigmoid(st["scores"][i]) for i in range(2)]
        return [gather, up, down]

    def add_to_stream(st):
        lane = lax.broadcasted_iota(I32, (D, 128), 1)
        for t, y in zip(st["toks"], st["y"]):
            n, at = locate(t)
            col = jnp.broadcast_to(y, (128, D)).astype(BF16).T.astype(F32)
            cur = xr[0, n]
            xr[0, n] = jnp.where(lane == at, cur + col, cur)

    def add_to_output(st):
        dma(wait=out_cp(1))()
        row = lax.broadcasted_iota(I32, (16, 128), 0)
        groups = [t // 16 for t in st["toks"]]
        patches = []
        for i, (t, y) in enumerate(zip(st["toks"], st["y"])):
            rows = pl.ds(pl.multiple_of(groups[i] * 16, 16), 16)
            for c in range(4):
                cur = xout[c, rows, :].astype(F32)
                new = jnp.where(row == t % 16, cur + y[:, 128 * c:128 * c + 128], cur)
                xout[c, rows, :] = new.astype(BF16)
            patches.append(copies([(xout.at[c, rows], out_hbm.at[rows, tiles(c)]) for c in range(4)], 4 * i))
        dma(start=patches[0])()
        pl.when(groups[0] != groups[1])(dma(patches[1], patches[1]))
        dma(wait=patches[0])()

    def run(plan, order, stages=(), keep=True, emit=True, reuse=None):
        def pos(i):
            return order[i] if i < NJ else i - NJ

        tasks = dict(
            X=load_x, Q=project_q, O=project_o, A=attend, C=clamp_v, U=layout_ffn,
            W=lambda t: layout_qkv(t) if t < 3 else layout_out(),
            R=lambda i: norm(i, order[i] if i < NJ else i),
            K=lambda i: project_kv(i, pos(i), 0, 1, i == reuse),
            V=lambda i: project_kv(i, pos(i), 1, 2),
            B=lambda i: project_kv(i, pos(i), 0, 2),
            P=lambda n: post(n, keep, emit),
            S=lambda i: _once(stages[i]))
        tick(None)
        pace["due"].clear()
        for group in plan:
            if group in (DENSE, LIGHT):
                pace["light"] = group == LIGHT
                continue
            streams = []
            for names in group:
                todo = [tasks[name[0]](int(name[1:])) for name in names.split() if name != "."]
                if names.endswith("."):
                    idle = COST["idle"] * sum(cost for _, cost in todo)
                    todo.append((iter([idle]), idle))
                streams.append(todo)
            _interleave(streams)

    def middle():
        order, st = {}, {}

        def choose():
            a, b = [(t // 2) % NJ for t in top2(NJ)[0]]
            b = jnp.where(a == b, (a + 1) % NJ, b)
            lo, hi = jnp.minimum(a, b), jnp.maximum(a, b)
            for i in range(NJ - 2):
                n = i + (i >= lo).astype(I32)
                order[i] = n + (n >= hi).astype(I32)
            order[NJ - 2], order[NJ - 1] = lo, hi

        dma(wait=ffn_cp)()
        run(MIDDLE, order, [choose, lambda: fence(wgu, pace["token"])] + route_stages(st)
            + [lambda: add_to_stream(st)], emit=False)
        return order[NJ - 2], order[NJ - 1]

    def shared(layer, tail):
        run(SHARED, {NJ - 2: tail[0], NJ - 1: tail[1]})
        return lax.cond(layer == 0, middle, lambda: tail)

    run(FIRST, list(range(NJ)), [
        dma([head_cp[0], w_cp[1], head_cp[1]], head_cp[:1]),
        dma(w_cp[2:], [w_cp[1], head_cp[1]]),
        dma(x_cp[0], w_cp[2:]),
        dma(x_cp[1] + w_cp[:1] + wo_cp, x_cp[0]),
        dma(ffn_cp, x_cp[1] + w_cp[:1] + wo_cp)], reuse=0)
    lax.fori_loop(0, 2, shared, (jnp.int32(NJ - 2), jnp.int32(NJ - 1)))
    st = {}
    run(LAST, None, [dma(out_cp(0, zero)), dma(out_cp(1), out_cp(0))] + route_stages(st)
        + [lambda: add_to_output(st)], keep=False)


@jax.jit
def pallas_interleave_layers__sliding_local_dilated__moe_arch_mod__prompt_kernel(
    A_x: jax.Array,
    A_wqkv: jax.Array,
    A_wo: jax.Array,
    B_x: jax.Array,
    B_w_r: jax.Array,
    B_w_gate: jax.Array,
    B_w_up: jax.Array,
    B_w_down: jax.Array,
):
    del B_x
    hbm = pl.BlockSpec(memory_space=pl.ANY)
    V = pltpu.VMEM
    block, weight = V((1, D + 8, 128), F32), V((1, D // 2 + 8, D), U32)

    def blocks(n):
        return V((1, n + 1, D, 128), F32)

    scratch = [
        V((64, 16, D), BF16), V((4, S, 128), BF16), V((4, S, 128), BF16),
        V((3, D, D), BF16), V((4, D, 128), BF16), V((D,), BF16),
        V((F, D), BF16), V((F, D), BF16), V((F, D), BF16),
        [weight] * 3, [weight] * 2, block, V((2, D // 2 + 8, FP), U32),
        blocks(NB), [block] * 6, blocks(NJ), [block] * NJ, blocks(NB),
        [blocks(2 * NB)] * 2, [block] * 3, [block] * 3, block, block,
        V((NB + 6, 8, 128), F32), V((NB, 128), F32),
        pltpu.SemaphoreType.DMA((21,)), pltpu.SemaphoreType.REGULAR,
    ]
    out = pl.pallas_call(
        _kernel,
        out_shape=jax.ShapeDtypeStruct((S, D), BF16),
        in_specs=[hbm] * 8,
        out_specs=hbm,
        scratch_shapes=scratch,
        compiler_params=pltpu.CompilerParams(vmem_limit_bytes=64 * 1024 * 1024),
    )(A_x.reshape(S, D), A_x.reshape(S // 16, 16, D), A_wqkv, A_wo, B_w_r,
      B_w_gate.T, B_w_up.T, B_w_down)
    return out.reshape(1, S, D)
```

```python
import jax
import jax.numpy as jnp
from jax import lax
import jax.experimental.pallas as pl
import jax.experimental.pallas.tpu as pltpu

S, D, F = 2048, 512, 1376
FP = 1408
NJ = 8
NB = 2 * NJ
EPS = 1e-5
NEG = -1e9
F32, BF16, U32, I32 = jnp.float32, jnp.bfloat16, jnp.uint32, jnp.int32
NT = (((1,), (1,)), ((), ()))
SLAB = 32
R = 64

FIRST = (
    dict(idle=0.2, qk=16, sm=72, pv=31, p1=52, p2=20, p3=14, r1=8, r2=24, r3=30, r4=20, light=True),
    ("X0 R0",), ("S0",), ("W1",), ("S1",), ("X1 R1",), ("Y2",), ("K0 K1 V0",), ("S2",),
    ("X2 R2",), ("V1",), ("X3 X4 X5 X6 X7",), ("K2 V2", "R3 R4 ."), ("K3 V3", "R5 ."), ("S3",),
    ("X8 X9 X10 X11 X12 X13 X14 X15",), ("K4 V4",), ("S4",), ("Y0",), ("W3",), ("K5 V5", "R6 ."),
)
SHARED = (
    dict(idle=0.2, qk=16, sm=24, pv=28, p1=32, p2=20, p3=20, r1=8, r2=24, r3=60, r4=20, light=True),
    ("V6 K6 V7", "R7 R9 R8 ."), ("K7 Q0", "C0"), ("B8 Q1", "R10 A0"), ("B9 Q2 O0", "R11", "A1"),
    ("B10 Q3 O1", "R12", "P0", "A2"), ("B11 Q4 O2", "R13", "P1", "A3"),
    ("B12 Q5 O3", "R14", "P2", "A4"), ("B13 Q6 O4", "R15", "P3", "A5"), ("B14 Q7 O5", "P4", "A6"),
    ("B15 Q8 O6", "P5 .", "A7"),
)
MIDDLE = (
    dict(idle=0.7, qk=18, sm=72, pv=31, p1=52, p2=40, p3=30, r1=14, r2=32, r3=60, r4=20, light=False),
    ("U0 U1",), ("Q9 O7", "P6 A8"), ("Q10 O8", "P7 A9"), ("S0",), ("Q11 O9", "P8 A10"),
    ("Q12 O10", "P9 A11"),
    dict(idle=0.7, qk=16, sm=72, pv=31, p1=32, p2=80, p3=30, r1=8, r2=24, r3=30, r4=20, light=True),
    ("Q13 O11 K0", "R0 P10", "A12"), ("Q14 V0 O12", "P11 R1", "A13"), ("S1",),
    ("Q15 O13 K1", "P12 R2", "A14"), ("V1 O14", "P13 R3", "A15"), ("K2 O15", "P14"),
    ("V2", "P15 ."), ("K3", "R4"), ("V3",), ("S2",), ("K4", "R5"), ("S3",), ("S4",), ("V4",),
    ("S5",), ("K5 V5", "R6 ."),
)
LAST = (
    dict(idle=0.1, qk=16, sm=96, pv=31, p1=52, p2=80, p3=30, r1=8, r2=24, r3=30, r4=12, light=False),
    ("Q9 O7", "P6 A8"), ("Q10 O8", "P7 A9"), ("S0",), ("Q11 O9 Q12", "A10 A11"),
    ("O10 Q13", "P8 A12"), ("O11 Q14", "P9 A13"), ("O12 Q15", "P10 A14"),
    ("O13 O14", "A15 P11 P12"), ("O15", "P13 P14 ."), ("P15",), ("S1",), ("S2",), ("S3",),
    ("S4",), ("S5",),
)


def _unpack(u):
    return pltpu.bitcast(u, BF16)


def _fold(x):
    parts = [x[8 * i:8 * i + 8] for i in range(x.shape[0] // 8)]
    while len(parts) > 1:
        parts = [parts[i] + parts[i + 1] for i in range(0, len(parts), 2)]
    return parts[0]


def _acc(a, b):
    return b if a is None else a + b


def _mean(partial):
    return jnp.sum(partial, axis=0, keepdims=True) * (1.0 / D)


def _rows(row):
    return jnp.broadcast_to(row, (R, 128))


def _once(fn):
    def gen():
        fn()
        yield 0
    return gen(), 0


def _interleave(streams):
    def chain(tasks):
        for gen, _ in tasks:
            yield from gen
    live = [[chain(t), 0, max(1, sum(c for _, c in t))] for t in reversed(streams)]
    while live:
        st = min(live, key=lambda e: e[1] / e[2])
        cost = next(st[0], None)
        if cost is None:
            live = [e for e in live if e is not st]
        else:
            st[1] += cost


def _kernel(x_hbm, x3_hbm, wqkv_hbm, wo_hbm, wr_hbm, wg_hbm, wu_hbm, wd_hbm, out_hbm,
            xhead, xin, xout, wqkv, wo, wr, wg, wu, wd, wt, wot, wrc, wgu, wtmp,
            xr, xo, xq, xn, kv, qs, os_, ca, v00, stat, r_ref, patch, sems):
    pace = dict(token=None, seen=set(), light=True, due=[])

    def fence(ref, val):
        if val.dtype != ref.dtype:
            val = pltpu.bitcast(val, ref.dtype)
        mid = tuple(n - 1 for n in ref.shape[1:-2])
        ref[(zero,) + mid + (pl.ds(ref.shape[-2] - 8, 8), pl.ds(0, 128))] = val

    def tick(val):
        pace["token"] = val
        pace["seen"].clear()

    def gate(ref, after=None):
        val = None if id(ref) in pace["seen"] else pace["token"]
        if after is not None and pace["light"]:
            val = _acc(val, after)
        if val is not None:
            fence(ref, val)
            pace["seen"].add(id(ref))

    def copies(pairs, sem):
        return [pltpu.make_async_copy(src, dst, sems.at[sem]) for src, dst in pairs]

    def tiles(c):
        return pl.ds(128 * c, 128)

    def half(s):
        return pl.ds(S // 2 * s, S // 2)

    x_cp = [copies([(x_hbm.at[half(s), tiles(c)], xin.at[c, half(s)]) for c in range(4)], s)
            for s in range(2)]
    head_cp = [copies([(x3_hbm.at[pl.ds(0, 64), pl.ds(2 * j, 2)], xhead.at[:, pl.ds(2 * j, 2)])], 2 + j)
               for j in range(2)]
    w_cp = [copies([(wqkv_hbm.at[:, pl.ds(D * t, D)], wqkv.at[t])], 4 + t) for t in range(3)]
    wo_cp = copies([(wo_hbm.at[:, tiles(c)], wo.at[c, pl.ds(0, D)]) for c in range(4)] + [(wr_hbm, wr)], 4)
    ffn_cp = copies([(wg_hbm, wg), (wu_hbm, wu), (wd_hbm, wd)], 5)

    def out_cp(s, z=0):
        return copies([(xout.at[c + z, half(s)], out_hbm.at[half(s), tiles(c)]) for c in range(4)], s)

    def dma(start=(), wait=()):
        def run():
            for cp in start:
                cp.start()
            for cp in wait:
                cp.wait()
            if wait:
                tick(None)
        return run

    dma(head_cp[0] + w_cp[1] + head_cp[1], head_cp[0])()
    word = pltpu.bitcast(xhead.bitcast(U32)[pl.ds(0, 8), 0, tiles(0)], I32) & 255
    zero = ((word * (word + 1)) & 1)[0, 0]

    def layout_qkv(t):
        def gen():
            a = lax.broadcasted_iota(I32, (128, 128), 0)
            b = lax.broadcasted_iota(I32, (128, 128), 1)
            perm = jnp.where(b == (a % 8) * 16 + a // 8, 1.0, 0.0).astype(BF16)
            for g in range(4):
                w = lax.dot_general(perm, wqkv[t, :, tiles(g)], NT, preferred_element_type=F32)
                wt[t][0, pl.ds(64 * g, 64), :] = pltpu.bitcast(w.astype(BF16), U32)
                tick(w[-8:, -128:])
                if g == 3:
                    fence(wt[t], pace["token"])
                yield 128
        return gen(), 512

    def layout_qkv_vpu(t):
        def gen():
            for g in range(4):
                for c in range(4):
                    wtmp[c, pl.ds(64 * g, 64), :] = pltpu.bitcast(wqkv[t, tiles(c), tiles(g)].T, U32)
                    yield 8
            for g in range(4):
                for c in range(4):
                    rows = []
                    for d2 in range(8):
                        u = wtmp[c, pl.ds(64 * g + d2, 8, stride=8), :]
                        rows += [u << 16, u & jnp.uint32(0xFFFF0000)]
                    w = pltpu.bitcast(jnp.concatenate(rows, axis=0), F32)
                    w = w * 0.25 if t == 0 else w
                    wt[t][0, pl.ds(64 * g, 64), tiles(c)] = pltpu.bitcast(w.astype(BF16), U32)
                    if (g, c) == (3, 3):
                        fence(wt[t], w[:8])
                    yield 24
        return gen(), 512

    def layout_out():
        def gen():
            wrc[0, pl.ds(0, D), :] = jnp.broadcast_to(
                wr[...].astype(F32).reshape(1, D), (128, D)).astype(BF16).T.astype(F32)
            for c in range(4):
                for g in range(4):
                    rows = []
                    for d2 in range(8):
                        u = wo.bitcast(U32)[c, pl.ds(64 * g + d2, 8, stride=8), :]
                        rows += [u << 16, u & jnp.uint32(0xFFFF0000)]
                    w = pltpu.bitcast(jnp.concatenate(rows, axis=0), F32)
                    w = pltpu.bitcast(w.astype(BF16).T, U32)
                    for ref in wot:
                        ref[0, pl.ds(64 * c, 64), tiles(g)] = w
                    yield 32
        return gen(), 512

    def layout_ffn(i):
        def run():
            for f in range(FP // 128):
                rows = min(128, F - 128 * f)
                for c in range(4):
                    w = (wg, wu)[i][pl.ds(128 * f, rows), tiles(c)]
                    if rows < 128:
                        w = jnp.concatenate([w, jnp.zeros((128 - rows, 128), BF16)], axis=0)
                    wgu[i, pl.ds(64 * c, 64), tiles(f)] = pltpu.bitcast(w.T, U32)
        return _once(run)

    def block_rows(n):
        return pl.ds(S // 4 * (n // NJ) + n % NJ, 64, stride=NJ)

    def load_x(n):
        cost = 128 if n < 2 else 24

        def gen():
            for c in range(4):
                if n < 2:
                    u = xhead.bitcast(U32)[:, n, tiles(c)]
                else:
                    u = xin.bitcast(U32)[c, block_rows(n), :]
                xr[0, n, tiles(c), :] = _unpack(u).T.astype(F32)
                yield cost
        return gen(), 4 * cost

    def norm(i, n):
        def gen():
            s = None
            for r0 in range(0, D, R):
                gate(xr)
                s = _acc(s, _fold(xr[0, n, pl.ds(r0, R), :]))
                yield pace["r1"]
            m, s = _rows(_mean(s)), None
            for r0 in range(0, D, R):
                gate(xr, m[:8] if r0 == R else None)
                c = xr[0, n, pl.ds(r0, R), :] - m
                ca[0, pl.ds(r0, R), :] = c
                s = _acc(s, _fold(c * c))
                yield pace["r2"]
            rs = _rows(lax.rsqrt(_mean(s) + EPS))
            yield pace["r3"]
            for r0 in range(0, D, R):
                gate(ca, rs[:8] if r0 == R else None)
                y = ca[0, pl.ds(r0, R), :] * rs
                xn[i % NJ][0, pl.ds(r0, R), :] = y
                if i < NJ:
                    xq[0, n, pl.ds(r0, R), :] = y
                if r0 + R == D:
                    fence(xn[i % NJ], rs[:8])
                yield pace["r4"]
        return gen(), 8 * (pace["r1"] + pace["r2"] + pace["r4"]) + pace["r3"]

    def project(weights, ref, idx, store, done=None):
        m = D * len(weights)

        def gen():
            lhs = jnp.concatenate([w[0, pl.ds(0, D // 2), :] for w in weights], axis=0)
            rhs = ref[idx + (pl.ds(0, D), slice(None))].astype(BF16)
            out = jnp.dot(_unpack(lhs), rhs, preferred_element_type=F32)
            for r0 in range(0, m, SLAB):
                store(r0, out[r0:r0 + SLAB])
                tick(out[r0 + SLAB - 8:r0 + SLAB])
                if r0 == 0:
                    fence(ref, pace["token"])
                if (r0 + SLAB) % D == 0:
                    fence(weights[r0 // D], pace["token"])
                if done and r0 + SLAB == m:
                    done()
                yield SLAB
        return gen(), m

    def project_kv(i, j, lo, hi):
        s = i // NJ

        def store(r0, val):
            lane = lax.broadcasted_iota(I32, val.shape, 1)
            is_v = lo + r0 // D
            rows, off = pl.ds(r0 % D, SLAB), NB * is_v
            kv[s][0, off + NJ + j, rows, :] = val
            if isinstance(j, int) and j == 0:
                return
            if s == 0:
                shifted = pltpu.roll(val, 2, 1)
            elif is_v:
                shifted = pltpu.roll(jnp.where(lane >= 126, kv[0][0, off + NJ + j, rows, :], val), 2, 1)
            else:
                shifted = jnp.where(lane < 2, kv[0][0, j, rows, :], pltpu.roll(val, 2, 1))
            kv[s][0, off + j, rows, :] = shifted
        return project(wt[1 + lo:1 + hi], xn[i % NJ], (0,), store)

    def clamp_v(_):
        def gen():
            lane = lax.broadcasted_iota(I32, (R, 128), 1)
            for r0 in range(0, D, R):
                v = kv[0][0, NB + NJ, pl.ds(r0, R), :]
                v00[0, pl.ds(r0, R), :] = jnp.where(lane == 0, v, pltpu.roll(v, 1, 1))
            yield 128
            for r0 in range(0, D, 16):
                gate(v00)
                v = v00[0, pl.ds(r0, 16), :]
                for j in range(1, NJ):
                    pltpu.store(kv[0].at[0, NB + j, pl.ds(r0, 16), :], v, mask=lane[:16] < 2)
                yield 16
        return gen(), 640

    def project_q(n):
        def store(r0, q):
            qs[n % 3][0, pl.ds(r0, SLAB), :] = q
        ref, idx = (xq, (0, n)) if n < NJ else (xn[n - NJ], (0,))
        return project(wt[:1], ref, idx, store, lambda: fence(qs[n % 3], pace["token"]))

    def attend(n):
        s, j = divmod(n, NJ)

        def gen():
            lane = lax.broadcasted_iota(I32, (8, 128), 1)
            for g in range(4):
                logit = [None] * NJ
                for d in range(16):
                    rows = pl.ds(128 * g + 8 * d, 8)
                    gate(kv[s])
                    q = qs[n % 3][0, rows, :]
                    for w in range(NJ):
                        logit[w] = _acc(logit[w], q * kv[s][0, NJ + j - w, rows, :])
                    yield pace["qk"]
                if s == 0:
                    for w in range(j + 1, NJ):
                        logit[w] = jnp.where(lane < 2, NEG, logit[w])
                top = logit
                while len(top) > 1:
                    top = [jnp.maximum(top[i], top[i + 1]) for i in range(0, len(top), 2)]
                e = [jnp.exp(a - top[0]) for a in logit]
                den = ((e[0] + e[1]) + (e[2] + e[3])) + ((e[4] + e[5]) + (e[6] + e[7]))
                inv = 1.0 / den
                yield pace["sm"]
                for d in range(16):
                    rows = pl.ds(128 * g + 8 * d, 8)
                    if d % 2 == 0:
                        gate(kv[s], den if d == 2 else None)
                    o = None
                    for w in range(NJ):
                        o = _acc(o, e[w] * kv[s][0, NB + NJ + j - w, rows, :])
                    os_[n % 3][0, rows, :] = o * inv
                    if (g, d) == (3, 15):
                        while pace["due"]:
                            o = o + pace["due"].pop()
                        fence(os_[n % 3], o)
                    if d % 2:
                        yield pace["pv"]
        return gen(), 4 * (16 * pace["qk"] + pace["sm"] + 8 * pace["pv"])

    def project_o(n):
        total = [None]

        def store(r0, y):
            x = xr[0, n, pl.ds(r0, SLAB), :] + y
            xo[n % 6][0, pl.ds(r0, SLAB), :] = x
            total[0] = _acc(total[0], _fold(x))

        def done():
            stat[NB + n] = jnp.broadcast_to(_mean(total[0]), (8, 128))
        return project([wot[n % 2]], os_[n % 3], (0,), store, done)

    def post(n, emit):
        def gen():
            m = jnp.concatenate([stat[NB + n]] * (R // 8), axis=0)
            s = t = None
            for r0 in range(0, D, R):
                rows = pl.ds(r0, R)
                gate(xo[n % 6], m[:8] if r0 == R else None)
                c = xo[n % 6][0, rows, :] - m
                s = _acc(s, _fold(c * c))
                t = _acc(t, _fold(c * wrc[0, rows, :]))
                yield pace["p1"]
            rs = lax.rsqrt(_mean(s) + EPS)
            r_ref[pl.ds(n, 1), :] = jnp.sum(t, axis=0, keepdims=True) * rs
            stat[n] = jnp.broadcast_to(rs / (rs + 1.0), (8, 128))
            fence(wrc, t)
            gain = _rows(rs)
            g1, g0 = gain + 1.0, gain * m
            yield pace["p2"]
            for c in range(4):
                gate(xo[n % 6], gain[:8] if c == 1 else None)
                ys = []
                for r0 in range(128 * c, 128 * c + 128, R):
                    x = xo[n % 6][0, pl.ds(r0, R), :]
                    ys.append(x * g1 - g0)
                    xr[0, n, pl.ds(r0, R), :] = ys[-1]
                    yield pace["p3"]
                if emit:
                    y = jnp.concatenate(ys, axis=0).astype(BF16)
                    xout.bitcast(U32)[c, block_rows(n), :] = pltpu.bitcast(y.T, U32)
            if emit and n < 11:
                seen = xout.bitcast(U32)[zero + 3, pl.ds(S // 4 * (n // NJ) + n % NJ, 1), :]
                pace["due"].append(pltpu.bitcast(seen, F32))
        return gen(), 8 * (pace["p1"] + pace["p3"]) + pace["p2"]

    def top2(blocks):
        r = r_ref[pl.ds(0, blocks), :]
        blk = lax.broadcasted_iota(I32, r.shape, 0)
        lane = lax.broadcasted_iota(I32, r.shape, 1)
        tid = ((blk // NJ) * 1024 + (lane // 2) * 16 + (blk % NJ) * 2 + lane % 2).astype(F32)
        none = float(2 * S)
        key = jnp.where(r != r, -jnp.inf, r)
        best = key == jnp.max(key, keepdims=True)
        first = jnp.min(jnp.where(best, tid, none), keepdims=True)
        tied = jnp.sum(jnp.where(best, 1.0, 0.0), keepdims=True) > 1.5
        runner = jnp.max(jnp.where(best, -jnp.inf, key), keepdims=True)
        second = jnp.min(jnp.where(tied, jnp.where(best & (tid != first), tid, none),
                                   jnp.where(~best & (key == runner), tid, none)), keepdims=True)
        toks = [jnp.clip(i.astype(I32)[0, 0], 0, S - 1) for i in (first, second)]
        return toks, [jnp.sum(jnp.where(tid == i, r, 0.0), keepdims=True) for i in (first, second)]

    def locate(t):
        return (t // 1024) * NJ + (t // 2) % NJ, ((t % 1024) // 16) * 2 + t % 2

    def route_stages(st):
        def gather():
            st["toks"], st["scores"] = top2(NB)
            row = lax.broadcasted_iota(I32, (16, 128), 0)
            lane = lax.broadcasted_iota(I32, (D, 128), 1)
            sel = None
            for i, t in enumerate(st["toks"]):
                n, at = locate(t)
                normed = (xr[0, n] - stat[NB + n][:1]) * stat[n][:1]
                col = jnp.where(lane == at, normed, 0.0).astype(BF16)
                pick = jnp.where(row == i, 1.0, 0.0).astype(BF16)
                sel = _acc(sel, lax.dot_general(pick, col, NT, preferred_element_type=F32))
            st["x"] = sel.astype(BF16)

        def up():
            g, u = [jnp.dot(st["x"], _unpack(wgu[i, pl.ds(0, D // 2), :]),
                            preferred_element_type=F32)[:8, :F] for i in range(2)]
            h = g * jax.nn.sigmoid(g) * u
            st["h"] = jnp.concatenate([h, h], axis=0).astype(BF16)

        def down():
            y = jnp.dot(st["h"], wd[...], preferred_element_type=F32)
            st["y"] = [y[i:i + 1] * jax.nn.sigmoid(st["scores"][i]) for i in range(2)]
        return [gather, up, down]

    def add_to_stream(st):
        lane = lax.broadcasted_iota(I32, (D, 128), 1)
        for t, y in zip(st["toks"], st["y"]):
            n, at = locate(t)
            col = jnp.broadcast_to(y, (128, D)).astype(BF16).T.astype(F32)
            cur = xr[0, n]
            xr[0, n] = jnp.where(lane == at, cur + col, cur)

    def add_to_output(st):
        row = lax.broadcasted_iota(I32, (16, D), 0)
        bases = [pl.multiple_of(t // 16 * 16, 16) for t in st["toks"]]
        for i, base in enumerate(bases):
            new = jnp.concatenate([xout[c, pl.ds(base, 16), :].astype(F32) for c in range(4)], axis=1)
            for t, y in zip(st["toks"], st["y"]):
                new = jnp.where(row + base == t, new + y, new)
            patch[i] = new.astype(BF16)
        one, two = [copies([(patch.at[i], out_hbm.at[pl.ds(base, 16)])], 2 + i)
                    for i, base in enumerate(bases)]
        dma(wait=out_cp(1))()
        dma(start=one)()
        pl.when(bases[0] != bases[1])(dma(two, two))
        dma(wait=one)()

    def run(plan, order, stages=(), emit=True):
        def pos(i):
            return order[i] if i < NJ else i - NJ

        tasks = dict(
            X=load_x, Y=layout_qkv_vpu, Q=project_q, O=project_o, A=attend, C=clamp_v, U=layout_ffn,
            W=lambda t: layout_qkv(t) if t < 3 else layout_out(),
            R=lambda i: norm(i, order[i] if i < NJ else i),
            K=lambda i: project_kv(i, pos(i), 0, 1),
            V=lambda i: project_kv(i, pos(i), 1, 2),
            B=lambda i: project_kv(i, pos(i), 0, 2),
            P=lambda n: post(n, emit),
            S=lambda i: _once(stages[i]))
        tick(None)
        pace["due"].clear()
        for group in plan:
            if isinstance(group, dict):
                pace.update(group)
                continue
            streams = []
            for names in group:
                todo = [tasks[name[0]](int(name[1:])) for name in names.split() if name != "."]
                if names.endswith("."):
                    idle = pace["idle"] * sum(cost for _, cost in todo)
                    todo.append((iter([idle]), idle))
                streams.append(todo)
            _interleave(streams)

    def middle():
        order, st = {}, {}

        def choose():
            a, b = [(t // 2) % NJ for t in top2(NJ)[0]]
            b = jnp.where(a == b, (a + 1) % NJ, b)
            lo, hi = jnp.minimum(a, b), jnp.maximum(a, b)
            for i in range(NJ - 2):
                n = i + (i >= lo).astype(I32)
                order[i] = n + (n >= hi).astype(I32)
            order[NJ - 2], order[NJ - 1] = lo, hi

        dma(wait=ffn_cp)()
        run(MIDDLE, order, [choose, lambda: fence(wgu, pace["token"])] + route_stages(st)
            + [lambda: add_to_stream(st)], emit=False)
        return order[NJ - 2], order[NJ - 1]

    def shared(layer, tail):
        run(SHARED, {NJ - 2: tail[0], NJ - 1: tail[1]})
        return lax.cond(layer == 0, middle, lambda: tail)

    run(FIRST, list(range(NJ)), [
        dma(w_cp[2], w_cp[1]),
        dma(x_cp[0], w_cp[2] + head_cp[1]),
        dma(x_cp[1], x_cp[0]),
        dma(w_cp[0] + wo_cp, x_cp[1]),
        dma(ffn_cp, w_cp[0] + wo_cp)])
    lax.fori_loop(0, 2, shared, (jnp.int32(NJ - 2), jnp.int32(NJ - 1)))
    st = {}
    run(LAST, None, [dma(out_cp(0, zero)), dma(out_cp(1), out_cp(0))] + route_stages(st)
        + [lambda: add_to_output(st)])


@jax.jit
def pallas_interleave_layers__sliding_local_dilated__moe_arch_mod__prompt_kernel(
    A_x: jax.Array,
    A_wqkv: jax.Array,
    A_wo: jax.Array,
    B_x: jax.Array,
    B_w_r: jax.Array,
    B_w_gate: jax.Array,
    B_w_up: jax.Array,
    B_w_down: jax.Array,
):
    del B_x
    hbm = pl.BlockSpec(memory_space=pl.ANY)
    V = pltpu.VMEM
    block, weight = V((1, D + 8, 128), F32), V((1, D // 2 + 8, D), U32)

    def blocks(n):
        return V((1, n + 1, D, 128), F32)

    scratch = [
        V((64, 16, D), BF16), V((4, S + 16, 128), BF16), V((4, S + 16, 128), BF16),
        V((3, D, D), BF16), V((4, D + 16, 128), BF16), V((D,), BF16),
        V((F, D), BF16), V((F, D), BF16), V((F, D), BF16),
        [weight] * 3, [weight] * 2, block,
        V((2, D // 2 + 8, FP), U32), V((4, D // 2 + 8, 128), U32),
        blocks(NB), [block] * 6, blocks(NJ), [block] * NJ,
        [blocks(2 * NB)] * 2, [block] * 3, [block] * 3, block, block,
        V((2 * NB, 8, 128), F32), V((NB, 128), F32), V((2, 16, D), BF16),
        pltpu.SemaphoreType.DMA((7,)),
    ]
    out = pl.pallas_call(
        _kernel,
        out_shape=jax.ShapeDtypeStruct((S, D), BF16),
        in_specs=[hbm] * 8,
        out_specs=hbm,
        scratch_shapes=scratch,
        compiler_params=pltpu.CompilerParams(vmem_limit_bytes=64 * 1024 * 1024),
    )(A_x.reshape(S, D), A_x.reshape(S // 16, 16, D), A_wqkv, A_wo, B_w_r,
      B_w_gate.T, B_w_up.T, B_w_down)
    return out.reshape(1, S, D)
```
